```python
import jax
import jax.numpy as jnp

def _softmax(x, axis=-1):
    return jax.nn.softmax(x, axis=axis)

def _gelu(x):
    return jax.nn.gelu(x, approximate=True)

def _silu(x):
    return jax.nn.silu(x)

def _sigmoid(x):
    return jax.nn.sigmoid(x)

def _layernorm(x, axis=-1, eps=1e-05):
    m = jnp.mean(x, axis=axis, keepdims=True)
    v = jnp.var(x, axis=axis, keepdims=True)
    return (x - m) / jnp.sqrt(v + eps)

def _scatter_add(tgt, idx, src, axis=0):
    return tgt.at[idx].add(src)

def _segment_sum(src, seg, n):
    return jax.ops.segment_sum(src, seg, n)

class _Rng:

    def __init__(self, key):
        self._k = key

    def _next(self):
        self._k, sub = jax.random.split(self._k)
        return sub

    def normal(self, shape):
        return jax.random.normal(self._next(), shape, dtype=jnp.bfloat16)

    def randint(self, lo, hi, shape):
        return jax.random.randint(self._next(), shape, lo, hi, dtype=jnp.int32)

    def uniform(self, shape, lo=0.0, hi=1.0):
        return jax.random.uniform(self._next(), shape, jnp.bfloat16, lo, hi)

    def permutation(self, n):
        return jax.random.permutation(self._next(), n)
kernel_name = 'adaLN_cond__gqa_block_cached__moe_arch_mod__decode'

def setup_inputs():
    _rng = _Rng(jax.random.key(int.from_bytes(__import__("os").urandom(4), "little")))
    _w = lambda a: (lambda t: t.astype(jnp.bfloat16) if jnp.issubdtype(t.dtype, jnp.floating) else t)(jnp.asarray(a))

    def _A_setup():
        B, Sq, D = (4, 1, 512)
        Hq, Hkv, Sk, Dh = (32, 32, 8192, 128)
        assert Hq % Hkv == 0, (Hq, Hkv)
        return {'x': _w((lambda *s: _rng.normal(s) * 0.05)(B, Sq, D)), 'k_cache': _w((lambda *s: _rng.normal(s) * 0.05)(B, Hkv, Sk, Dh)), 'v_cache': _w((lambda *s: _rng.normal(s) * 0.05)(B, Hkv, Sk, Dh)), 'wq': _w((lambda *s: _rng.normal(s) * 0.05)(D, Hq * Dh) * D ** (-0.5)), 'wo': _w((lambda *s: _rng.normal(s) * 0.05)(Hq * Dh, D) * (Hq * Dh) ** (-0.5))}
    _A_in = _A_setup()

    def _B_setup():
        B, S, D, F, C = (4, 1, 512, 1376, 1)
        return {'x': _w((lambda *s: _rng.normal(s) * 0.05)(B, S, D)), 'w_r': _w((lambda *s: _rng.normal(s) * 0.05)(D)), 'w_gate': _w((lambda *s: _rng.normal(s) * 0.05)(D, F)), 'w_up': _w((lambda *s: _rng.normal(s) * 0.05)(D, F)), 'w_down': _w((lambda *s: _rng.normal(s) * 0.05)(F, D))}
    _B_in = _B_setup()
    return {'A_x': _A_in['x'], 'A_k_cache': _A_in['k_cache'], 'A_v_cache': _A_in['v_cache'], 'A_wq': _A_in['wq'], 'A_wo': _A_in['wo'], 'B_x': _B_in['x'], 'B_w_r': _B_in['w_r'], 'B_w_gate': _B_in['w_gate'], 'B_w_up': _B_in['w_up'], 'B_w_down': _B_in['w_down'], 'c': _w((lambda *s: _rng.normal(s) * 0.05)(4, 512)), 'w_mod': _w((lambda *s: _rng.normal(s) * 0.05)(512, 6 * 512) * 512 ** (-0.5))}

def reference(A_x, A_k_cache, A_v_cache, A_wq, A_wo, B_x, B_w_r, B_w_gate, B_w_up, B_w_down, c, w_mod):

    def _A_ref(x, k_cache, v_cache, wq, wo):
        B, Sq, D = x.shape
        Hq, Dh = (32, 128)
        Hkv = k_cache.shape[1]
        rep = Hq // Hkv
        q = (lambda x, *d: x.transpose(*d))((x @ wq).reshape(B, Sq, Hq, Dh), 0, 2, 1, 3)
        k = jnp.repeat(k_cache, rep, axis=1)
        v = jnp.repeat(v_cache, rep, axis=1)
        scores = jnp.einsum('bhqd,bhkd->bhqk', q, k) * Dh ** (-0.5)
        p = _softmax(scores, axis=-1)
        o = jnp.einsum('bhqk,bhkd->bhqd', p, v)
        return (lambda x, *d: x.transpose(*d))(o, 0, 2, 1, 3).reshape(B, Sq, Hq * Dh) @ wo

    def _B_ref(x, w_r, w_gate, w_up, w_down):
        B, S, D = x.shape
        C = 1
        r = x @ w_r
        idx = jnp.argsort(-r, axis=-1)[:, :C]
        idx_e = jnp.repeat(idx.reshape(B, C, 1), D, axis=2)
        x_sel = jnp.take_along_axis(x, idx_e, axis=1)
        g = _silu(x_sel @ w_gate)
        u = x_sel @ w_up
        y = g * u @ w_down
        r_sel = _sigmoid(jnp.take_along_axis(r, idx, axis=1))
        y = y * r_sel.reshape(B, C, 1)
        b_off = (jnp.arange(B) * S).reshape(B, 1)
        flat_idx = (idx + b_off).reshape(B * C)
        zero = (x * 0.0).reshape(B * S, D)
        upd = _scatter_add(zero, flat_idx, y.reshape(B * C, D), axis=0)
        return x + upd.reshape(B, S, D)
    x = A_x
    mod = (_silu(c) @ w_mod).reshape(c.shape[0], 6, 1, -1)
    sa, ca, ga, sb, cb, gb = (mod[:, 0].copy(), mod[:, 1].copy(), mod[:, 2].copy(), mod[:, 3].copy(), mod[:, 4].copy(), mod[:, 5].copy())
    h = _layernorm(x, axis=-1) * (1 + ca) + sa
    x = x + ga * _A_ref(h, A_k_cache, A_v_cache, A_wq, A_wo)
    h = _layernorm(x, axis=-1) * (1 + cb) + sb
    x = x + gb * _B_ref(h, B_w_r, B_w_gate, B_w_up, B_w_down)
    return x
```

```python
import jax
import jax.numpy as jnp
from jax import lax
import jax.experimental.pallas as pl
import jax.experimental.pallas.tpu as pltpu

f32 = jnp.float32
bf16 = jnp.bfloat16
LANES = 128
N_SLOTS = 4
EPS = 1e-5
NT_DIMS = (((1,), (1,)), ((), ()))


def _layernorm(x):
    xc = x - jnp.mean(x, axis=-1, keepdims=True)
    var = jnp.mean(xc * xc, axis=-1, keepdims=True)
    return xc / jnp.sqrt(var + EPS)


def _dot(a, w):
    return jnp.dot(a, w, preferred_element_type=f32)


def _dot_nt(a, w):
    return lax.dot_general(a, w, NT_DIMS, preferred_element_type=f32)


@jax.jit
def pallas_adaLN_cond__gqa_block_cached__moe_arch_mod__decode_kernel(
    A_x: jax.Array,
    A_k_cache: jax.Array,
    A_v_cache: jax.Array,
    A_wq: jax.Array,
    A_wo: jax.Array,
    B_x: jax.Array,
    B_w_r: jax.Array,
    B_w_gate: jax.Array,
    B_w_up: jax.Array,
    B_w_down: jax.Array,
    c: jax.Array,
    w_mod: jax.Array,
):
    del B_x
    B, SQ, D = A_x.shape
    _, H, SK, DH = A_k_cache.shape
    F = B_w_gate.shape[1]
    assert SQ == 1 and A_wq.shape == (D, H * DH) and w_mod.shape == (D, 6 * D)
    assert D % LANES == 0 and DH == LANES
    n_steps = B * H
    scale = DH ** -0.5
    gb_cols = ((0, D - LANES), (D - LANES, D))

    def kernel(x_hbm, k_hbm, v_hbm, wq_hbm, wo_hbm, wr_hbm, wg_hbm, wu_hbm, wd_hbm, c_hbm, wm_hbm,
               out_ref,
               kbuf, vbuf, wq_v, wo_v, wm_v, wg_v, wu_v, wd_v, x_v, c_v, wr_v, q_v, gb0_v, gb1_v,
               ksem, vsem, wsem):
        gb_v = (gb0_v, gb1_v)

        def kv_start(s, slot):
            h, b = s // B, s % B
            pltpu.make_async_copy(k_hbm.at[b, h], kbuf.at[slot], ksem.at[slot]).start()
            pltpu.make_async_copy(v_hbm.at[b, h], vbuf.at[slot], vsem.at[slot]).start()

        def k_wait(slot):
            pltpu.make_async_copy(kbuf.at[slot], kbuf.at[slot], ksem.at[slot]).wait()

        def v_wait(slot):
            pltpu.make_async_copy(vbuf.at[slot], vbuf.at[slot], vsem.at[slot]).wait()

        cp_c = pltpu.make_async_copy(c_hbm, c_v, wsem.at[0])
        cp_x = pltpu.make_async_copy(x_hbm, x_v, wsem.at[1])
        cp_wm = pltpu.make_async_copy(wm_hbm.at[:, 0:5 * D], wm_v, wsem.at[2])
        cp_wq = pltpu.make_async_copy(wq_hbm, wq_v, wsem.at[3])
        cp_wo = pltpu.make_async_copy(wo_hbm, wo_v, wsem.at[4])
        cp_wr = pltpu.make_async_copy(wr_hbm, wr_v, wsem.at[5])
        cp_wg = pltpu.make_async_copy(wg_hbm, wg_v, wsem.at[6])
        cp_wu = pltpu.make_async_copy(wu_hbm, wu_v, wsem.at[7])
        cp_wd = pltpu.make_async_copy(wd_hbm, wd_v, wsem.at[8])
        cp_gb = [pltpu.make_async_copy(wm_hbm.at[:, 5 * D + lo:5 * D + hi], gb_v[i], wsem.at[9 + i])
                 for i, (lo, hi) in enumerate(gb_cols)]

        cp_wm.start()
        cp_c.start()
        cp_x.start()
        cp_wq.start()
        for s in range(N_SLOTS):
            kv_start(s, s)
        cp_wo.start()
        cp_wr.start()

        cp_c.wait()
        cp_wm.wait()
        silu_c = jax.nn.silu(c_v[...].astype(f32)).astype(bf16)
        mod = _dot(silu_c, wm_v[...])
        sa, ca, ga, sb, cb = (mod[:, i * D:(i + 1) * D] for i in range(5))
        cp_x.wait()
        x0 = x_v[...].astype(f32)
        h1 = (_layernorm(x0) * (1 + ca) + sa).astype(bf16)
        cp_wq.wait()
        q = _dot(h1, wq_v[...]).astype(bf16)
        for h in range(H):
            q_v[h] = q[:, h * DH:(h + 1) * DH]
        cp_wo.wait()

        batch_row = lax.broadcasted_iota(jnp.int32, (B, DH), 0)

        def head_step(s, carry):
            o_head, attn = carry
            slot = s % N_SLOTS
            h, b = s // B, s % B
            k_wait(slot)
            scores = _dot_nt(q_v[h], kbuf[slot])
            p = jnp.exp((scores - jnp.max(scores, axis=1, keepdims=True)) * scale)
            denom = jnp.sum(p, axis=1, keepdims=True)
            v_wait(slot)
            o = _dot(p.astype(bf16), vbuf[slot]) / denom

            @pl.when(s + N_SLOTS < n_steps)
            def _():
                kv_start(s + N_SLOTS, slot)

            @pl.when(s + N_SLOTS == n_steps)
            def _():
                for cp in (cp_wg, cp_wu, cp_wd, *cp_gb):
                    cp.start()

            o_head = jnp.where(batch_row == b, o, o_head)

            def project(attn):
                wo_h = wo_v[pl.ds(pl.multiple_of(h * DH, DH), DH), :]
                return attn + _dot(o_head.astype(bf16), wo_h)

            attn = lax.cond(b == B - 1, project, lambda attn: attn, attn)
            return o_head, attn

        _, attn = lax.fori_loop(
            0, n_steps, head_step, (jnp.zeros((B, DH), f32), jnp.zeros((B, D), f32)))

        x1 = x0 + ga * attn
        h2 = _layernorm(x1) * (1 + cb) + sb
        h2b = h2.astype(bf16)
        cp_wr.wait()
        w_r = wr_v[...].astype(f32)
        h2r = h2b.astype(f32)
        r = h2r[:, 0:LANES] * w_r[0:1, :]
        for i in range(1, D // LANES):
            r = r + h2r[:, i * LANES:(i + 1) * LANES] * w_r[i:i + 1, :]
        r_gate = jax.nn.sigmoid(jnp.sum(r, axis=1, keepdims=True))
        cp_wg.wait()
        g = _dot_nt(h2b, wg_v[...])
        cp_wu.wait()
        u = _dot_nt(h2b, wu_v[...])
        act = (jax.nn.silu(g) * u).astype(bf16)
        cp_wd.wait()
        y = _dot(act, wd_v[...]) * r_gate
        ffn = h2 + (h2 * 0.0 + y)
        for i, (lo, hi) in enumerate(gb_cols):
            cp_gb[i].wait()
            gb = _dot(silu_c, gb_v[i][...])
            out_ref[:, lo:hi] = (x1[:, lo:hi] + gb * ffn[:, lo:hi]).astype(out_ref.dtype)

    hbm = pl.BlockSpec(memory_space=pltpu.HBM)
    out = pl.pallas_call(
        kernel,
        in_specs=[hbm] * 11,
        out_specs=pl.BlockSpec(memory_space=pltpu.VMEM),
        out_shape=jax.ShapeDtypeStruct((B, D), A_x.dtype),
        scratch_shapes=[
            pltpu.VMEM((N_SLOTS, SK, DH), bf16),
            pltpu.VMEM((N_SLOTS, SK, DH), bf16),
            pltpu.VMEM((D, H * DH), bf16),
            pltpu.VMEM((H * DH, D), bf16),
            pltpu.VMEM((D, 5 * D), bf16),
            pltpu.VMEM((F, D), bf16),
            pltpu.VMEM((F, D), bf16),
            pltpu.VMEM((F, D), bf16),
            pltpu.VMEM((B, D), bf16),
            pltpu.VMEM((B, D), bf16),
            pltpu.VMEM((D // LANES, LANES), bf16),
            pltpu.VMEM((H, B, DH), bf16),
            *(pltpu.VMEM((D, hi - lo), bf16) for lo, hi in gb_cols),
            pltpu.SemaphoreType.DMA((N_SLOTS,)),
            pltpu.SemaphoreType.DMA((N_SLOTS,)),
            pltpu.SemaphoreType.DMA((9 + len(gb_cols),)),
        ],
        compiler_params=pltpu.CompilerParams(
            vmem_limit_bytes=64 * 1024 * 1024,
            disable_semaphore_checks=True,
        ),
    )(
        A_x.reshape(B, D),
        A_k_cache,
        A_v_cache,
        A_wq,
        A_wo,
        B_w_r.reshape(D // LANES, LANES),
        B_w_gate.T,
        B_w_up.T,
        B_w_down,
        c,
        w_mod,
    )
    return out.reshape(B, SQ, D)
```

```python
import jax
import jax.numpy as jnp
from jax import lax
import jax.experimental.pallas as pl
import jax.experimental.pallas.tpu as pltpu

f32 = jnp.float32
bf16 = jnp.bfloat16
LANES = 128
N_SLOTS = 4
EPS = 1e-5
NT_DIMS = (((1,), (1,)), ((), ()))


def _layernorm(x):
    xc = x - jnp.mean(x, axis=-1, keepdims=True)
    var = jnp.mean(xc * xc, axis=-1, keepdims=True)
    return xc / jnp.sqrt(var + EPS)


def _dot(a, w):
    return jnp.dot(a, w, preferred_element_type=f32)


def _dot_nt(a, w):
    return lax.dot_general(a, w, NT_DIMS, preferred_element_type=f32)


@jax.jit
def pallas_adaLN_cond__gqa_block_cached__moe_arch_mod__decode_kernel(
    A_x: jax.Array,
    A_k_cache: jax.Array,
    A_v_cache: jax.Array,
    A_wq: jax.Array,
    A_wo: jax.Array,
    B_x: jax.Array,
    B_w_r: jax.Array,
    B_w_gate: jax.Array,
    B_w_up: jax.Array,
    B_w_down: jax.Array,
    c: jax.Array,
    w_mod: jax.Array,
):
    del B_x
    B, SQ, D = A_x.shape
    _, H, SK, DH = A_k_cache.shape
    F = B_w_gate.shape[1]
    assert SQ == 1 and A_wq.shape == (D, H * DH) and w_mod.shape == (D, 6 * D)
    assert D % LANES == 0 and DH == LANES
    n_steps = B * H
    scale = DH ** -0.5
    n_tiles = F // LANES
    cuts = sorted({0, F, *(LANES * (n_tiles * k // 10) for k in (4, 7, 9))})
    wd_rows = tuple(zip(cuts[:-1], cuts[1:]))

    def kernel(x_hbm, k_hbm, v_hbm, wq_hbm, wo_hbm, wr_hbm, wg_hbm, wu_hbm, wd_hbm, c_hbm, wm_hbm,
               out_ref,
               kbuf, vbuf, wq_v, wo_v, wm_v, wg_v, wu_v, wd_v, x_v, c_v, wr_v, q_v,
               ksem, vsem, wsem):
        def kv_start(s, slot):
            h, b = s // B, s % B
            pltpu.make_async_copy(k_hbm.at[b, h], kbuf.at[slot], ksem.at[slot]).start()
            pltpu.make_async_copy(v_hbm.at[b, h], vbuf.at[slot], vsem.at[slot]).start()

        def k_wait(slot):
            pltpu.make_async_copy(kbuf.at[slot], kbuf.at[slot], ksem.at[slot]).wait()

        def v_wait(slot):
            pltpu.make_async_copy(vbuf.at[slot], vbuf.at[slot], vsem.at[slot]).wait()

        cp_c = pltpu.make_async_copy(c_hbm, c_v, wsem.at[0])
        cp_x = pltpu.make_async_copy(x_hbm, x_v, wsem.at[1])
        cp_wm = pltpu.make_async_copy(wm_hbm, wm_v, wsem.at[2])
        cp_wq = pltpu.make_async_copy(wq_hbm, wq_v, wsem.at[3])
        cp_wo = pltpu.make_async_copy(wo_hbm, wo_v, wsem.at[4])
        cp_wr = pltpu.make_async_copy(wr_hbm, wr_v, wsem.at[5])
        cp_wg = pltpu.make_async_copy(wg_hbm, wg_v, wsem.at[6])
        cp_wu = pltpu.make_async_copy(wu_hbm, wu_v, wsem.at[7])
        cp_wd = [pltpu.make_async_copy(wd_hbm.at[lo:hi], wd_v.at[lo:hi], wsem.at[8 + i])
                 for i, (lo, hi) in enumerate(wd_rows)]

        cp_wm.start()
        cp_c.start()
        cp_x.start()
        cp_wq.start()
        for s in range(N_SLOTS):
            kv_start(s, s)
        cp_wo.start()
        cp_wr.start()

        cp_c.wait()
        cp_wm.wait()
        silu_c = jax.nn.silu(c_v[...].astype(f32)).astype(bf16)
        mod = _dot(silu_c, wm_v[...])
        sa, ca, ga, sb, cb, gb = (mod[:, i * D:(i + 1) * D] for i in range(6))
        cp_x.wait()
        x0 = x_v[...].astype(f32)
        h1 = (_layernorm(x0) * (1 + ca) + sa).astype(bf16)
        cp_wq.wait()
        q = _dot(h1, wq_v[...]).astype(bf16)
        for h in range(H):
            q_v[h] = q[:, h * DH:(h + 1) * DH]
        cp_wo.wait()

        batch_row = lax.broadcasted_iota(jnp.int32, (B, DH), 0)

        def head_step(s, carry):
            o_head, attn = carry
            slot = s % N_SLOTS
            h, b = s // B, s % B
            k_wait(slot)
            scores = _dot_nt(q_v[h], kbuf[slot])
            p = jnp.exp((scores - jnp.max(scores, axis=1, keepdims=True)) * scale)
            denom = jnp.sum(p, axis=1, keepdims=True)
            v_wait(slot)
            o = _dot(p.astype(bf16), vbuf[slot]) / denom

            @pl.when(s + N_SLOTS < n_steps)
            def _():
                kv_start(s + N_SLOTS, slot)

            @pl.when(s + N_SLOTS == n_steps)
            def _():
                for cp in (cp_wg, cp_wu, *cp_wd):
                    cp.start()

            o_head = jnp.where(batch_row == b, o, o_head)

            def project(attn):
                wo_h = wo_v[pl.ds(pl.multiple_of(h * DH, DH), DH), :]
                return attn + _dot(o_head.astype(bf16), wo_h)

            attn = lax.cond(b == B - 1, project, lambda attn: attn, attn)
            return o_head, attn

        _, attn = lax.fori_loop(
            0, n_steps, head_step, (jnp.zeros((B, DH), f32), jnp.zeros((B, D), f32)))

        x1 = x0 + ga * attn
        h2 = _layernorm(x1) * (1 + cb) + sb
        h2b = h2.astype(bf16)
        cp_wr.wait()
        w_r = wr_v[...].astype(f32)
        h2r = h2b.astype(f32)
        r = h2r[:, 0:LANES] * w_r[0:1, :]
        for i in range(1, D // LANES):
            r = r + h2r[:, i * LANES:(i + 1) * LANES] * w_r[i:i + 1, :]
        r_gate = jax.nn.sigmoid(jnp.sum(r, axis=1, keepdims=True))
        cp_wg.wait()
        g = _dot_nt(h2b, wg_v[...])
        cp_wu.wait()
        u = _dot_nt(h2b, wu_v[...])
        act = (jax.nn.silu(g) * u).astype(bf16)
        out = x1 + gb * (h2 + h2 * 0.0)
        y_scale = gb * r_gate
        for cp, (lo, hi) in zip(cp_wd, wd_rows):
            cp.wait()
            out = out + y_scale * _dot(act[:, lo:hi], wd_v[lo:hi, :])
        out_ref[...] = out.astype(out_ref.dtype)

    hbm = pl.BlockSpec(memory_space=pltpu.HBM)
    out = pl.pallas_call(
        kernel,
        in_specs=[hbm] * 11,
        out_specs=pl.BlockSpec(memory_space=pltpu.VMEM),
        out_shape=jax.ShapeDtypeStruct((B, D), A_x.dtype),
        scratch_shapes=[
            pltpu.VMEM((N_SLOTS, SK, DH), bf16),
            pltpu.VMEM((N_SLOTS, SK, DH), bf16),
            pltpu.VMEM((D, H * DH), bf16),
            pltpu.VMEM((H * DH, D), bf16),
            pltpu.VMEM((D, 6 * D), bf16),
            pltpu.VMEM((F, D), bf16),
            pltpu.VMEM((F, D), bf16),
            pltpu.VMEM((F, D), bf16),
            pltpu.VMEM((B, D), bf16),
            pltpu.VMEM((B, D), bf16),
            pltpu.VMEM((D // LANES, LANES), bf16),
            pltpu.VMEM((H, B, DH), bf16),
            pltpu.SemaphoreType.DMA((N_SLOTS,)),
            pltpu.SemaphoreType.DMA((N_SLOTS,)),
            pltpu.SemaphoreType.DMA((8 + len(wd_rows),)),
        ],
        compiler_params=pltpu.CompilerParams(
            vmem_limit_bytes=64 * 1024 * 1024,
            disable_semaphore_checks=True,
        ),
    )(
        A_x.reshape(B, D),
        A_k_cache,
        A_v_cache,
        A_wq,
        A_wo,
        B_w_r.reshape(D // LANES, LANES),
        B_w_gate.T,
        B_w_up.T,
        B_w_down,
        c,
        w_mod,
    )
    return out.reshape(B, SQ, D)
```

```python
import jax
import jax.numpy as jnp
from jax import lax
import jax.experimental.pallas as pl
import jax.experimental.pallas.tpu as pltpu

f32 = jnp.float32
bf16 = jnp.bfloat16
LANES = 128
EPS = 1e-5
NT_DIMS = (((1,), (1,)), ((), ()))

HG = 4
SEGS = 2
ROWS = 64
N_SLOTS = 3
AHEAD = 16
TAIL_FIRST, TAIL_STEP = 64, 28


def _layernorm(x):
    xc = x - jnp.mean(x, axis=-1, keepdims=True)
    var = jnp.mean(xc * xc, axis=-1, keepdims=True)
    return xc / jnp.sqrt(var + EPS)


def _dot(a, w):
    return jnp.dot(a, w, preferred_element_type=f32)


def _dot_nt(a, w):
    return lax.dot_general(a, w, NT_DIMS, preferred_element_type=f32)


@jax.jit
def pallas_adaLN_cond__gqa_block_cached__moe_arch_mod__decode_kernel(
    A_x: jax.Array,
    A_k_cache: jax.Array,
    A_v_cache: jax.Array,
    A_wq: jax.Array,
    A_wo: jax.Array,
    B_x: jax.Array,
    B_w_r: jax.Array,
    B_w_gate: jax.Array,
    B_w_up: jax.Array,
    B_w_down: jax.Array,
    c: jax.Array,
    w_mod: jax.Array,
):
    del B_x
    B, SQ, D = A_x.shape
    _, H, SK, DH = A_k_cache.shape
    F = B_w_gate.shape[1]
    assert SQ == 1 and A_wq.shape == (D, H * DH) and w_mod.shape == (D, 6 * D)
    assert D % LANES == 0 and DH == LANES
    scale = DH ** -0.5

    seg = SK // SEGS
    n_grp = seg // ROWS
    n_steps = B * H
    n_grp_all = n_steps // HG * n_grp
    grp_step = n_grp // HG
    last_kv_step = -(-(n_grp_all - n_grp - AHEAD) // grp_step) - 1
    assert SK % (SEGS * ROWS) == 0 and H % HG == 0 and n_grp % HG == 0 and AHEAD <= n_grp

    cuts = sorted({0, F, *(LANES * (F // LANES * k // 10) for k in (4, 7, 9))})
    wd_rows = tuple(zip(cuts[:-1], cuts[1:]))

    def kernel(x_hbm, k_hbm, v_hbm, wq_hbm, wo_hbm, wr_hbm, wg_hbm, wu_hbm, wd_hbm, c_hbm, wm_hbm,
               out_ref,
               kbuf, vbuf, wq_v, wo_v, wm_v, wg_v, wu_v, wd_v, x_v, c_v, wr_v, q_v, o_v,
               ksem, vsem, wsem):
        C_SEM, X_SEM, WM_SEM, WQ_SEM, WO_SEM, WR_SEM, WG_SEM, WU_SEM, WD_SEM = range(9)

        def copy(src, dst, sem):
            return pltpu.make_async_copy(src, dst, sem)

        def wait_all(buf, sem):
            copy(buf, buf, sem).wait()

        def kv_issue(lo, hi):
            def group(u, _):
                blk = u // n_grp
                slot, hg, b = blk % N_SLOTS, blk // B, blk % B
                rows = pl.ds(pl.multiple_of(u % n_grp * ROWS, ROWS), ROWS)
                for j in range(HG):
                    segs = pl.ds((hg * HG + j) * SEGS, SEGS)
                    copy(k_hbm.at[b, segs, rows], kbuf.at[slot, j, :, rows], ksem.at[slot]).start(priority=0)
                    copy(v_hbm.at[b, segs, rows], vbuf.at[slot, j, :, rows], vsem.at[slot]).start(priority=1)
            lax.fori_loop(lo, hi, group, None)

        def wide_issue(src, dst, sem):
            def body(i, _):
                rows = pl.ds(pl.multiple_of(i * 8, 8), 8)
                for c0 in range(0, src.shape[2], 8 * LANES):
                    for p in range(2):
                        idx = (slice(2 * p, 2 * p + 2), rows, slice(c0, c0 + 8 * LANES))
                        copy(src.at[idx], dst.at[idx], sem).start(priority=p)
            lax.fori_loop(0, src.shape[1] // 8, body, None)

        tail = []
        for r0 in range(0, wo_hbm.shape[1], 16):
            for p in range(2):
                idx = (slice(2 * p, 2 * p + 2), slice(r0, r0 + 16))
                tail.append((copy(wo_hbm.at[idx], wo_v.at[idx], wsem.at[WO_SEM]), p))
        tail.append((copy(wr_hbm, wr_v, wsem.at[WR_SEM]), 0))
        for r0 in range(0, F, 32):
            rows = slice(r0, min(r0 + 32, F))
            tail.append((copy(wg_hbm.at[rows], wg_v.at[rows], wsem.at[WG_SEM]), 0))
            tail.append((copy(wu_hbm.at[rows], wu_v.at[rows], wsem.at[WU_SEM]), 1))
        for i, (lo, hi) in enumerate(wd_rows):
            for r0 in range(lo, hi, 32):
                rows = slice(r0, min(r0 + 32, hi))
                tail.append((copy(wd_hbm.at[rows], wd_v.at[rows], wsem.at[WD_SEM + i]), r0 // 32 % 2))
        tail_cuts = [0]
        for i in range(n_steps - last_kv_step):
            tail_cuts.append(min(len(tail), tail_cuts[-1] + (TAIL_STEP if i else TAIL_FIRST)))

        def tail_issue(lo, hi):
            for cp, queue in tail[lo:hi]:
                cp.start(priority=queue)

        wide_issue(wm_hbm, wm_v, wsem.at[WM_SEM])
        copy(c_hbm, c_v, wsem.at[C_SEM]).start(priority=0)
        copy(x_hbm, x_v, wsem.at[X_SEM]).start(priority=1)
        wide_issue(wq_hbm, wq_v, wsem.at[WQ_SEM])

        wait_all(wm_v, wsem.at[WM_SEM])
        wait_all(c_v, wsem.at[C_SEM])
        silu_c = jax.nn.silu(c_v[...].astype(f32)).astype(bf16)
        mod = _dot(silu_c, wm_v[...].reshape(D, 6 * D))
        sa, ca, ga, sb, cb, gb = (mod[:, i * D:(i + 1) * D] for i in range(6))
        wait_all(x_v, wsem.at[X_SEM])
        x0 = x_v[...].astype(f32)
        h1 = (_layernorm(x0) * (1 + ca) + sa).astype(bf16)

        kv_issue(0, n_grp // 2)
        o_v[...] = jnp.zeros_like(o_v)

        wait_all(wq_v, wsem.at[WQ_SEM])
        q = _dot(h1, wq_v[...].reshape(D, H * DH)).astype(bf16)
        for h in range(H):
            q_v[h] = q[:, h * DH:(h + 1) * DH]

        kv_issue(n_grp // 2, n_grp + AHEAD)

        batch_row = lax.broadcasted_iota(jnp.int32, (B, DH), 0)

        def head_step(s, _):
            blk, j = s // HG, s % HG
            slot, hg, b = blk % N_SLOTS, blk // B, blk % B
            h = hg * HG + j

            @pl.when(j == 0)
            def _():
                wait_all(kbuf.at[slot], ksem.at[slot])
                wait_all(vbuf.at[slot], vsem.at[slot])

            scores = _dot_nt(q_v[h], kbuf[slot, j].reshape(SK, DH))
            p = jnp.exp((scores - jnp.max(scores, axis=1, keepdims=True)) * scale)
            denom = jnp.sum(p, axis=1, keepdims=True)
            o = _dot(p.astype(bf16), vbuf[slot, j].reshape(SK, DH)) / denom
            o_v[h] = jnp.where(batch_row == b, o, o_v[h])

            lo = jnp.minimum(n_grp + AHEAD + grp_step * s, n_grp_all)
            kv_issue(lo, jnp.minimum(lo + grp_step, n_grp_all))

            for i in range(len(tail_cuts) - 1):
                @pl.when(s == last_kv_step + i)
                def _():
                    tail_issue(tail_cuts[i], tail_cuts[i + 1])

        lax.fori_loop(0, n_steps, head_step, None)
        tail_issue(tail_cuts[-1], len(tail))

        wait_all(wo_v, wsem.at[WO_SEM])
        o_all = jnp.concatenate([o_v[h] for h in range(H)], axis=1).astype(bf16)
        x1 = x0 + ga * _dot(o_all, wo_v[...].reshape(H * DH, D))
        h2 = _layernorm(x1) * (1 + cb) + sb
        h2b = h2.astype(bf16)
        wait_all(wr_v, wsem.at[WR_SEM])
        w_r = wr_v[...].astype(f32)
        h2r = h2b.astype(f32)
        r = h2r[:, 0:LANES] * w_r[0:1, :]
        for i in range(1, D // LANES):
            r = r + h2r[:, i * LANES:(i + 1) * LANES] * w_r[i:i + 1, :]
        r_gate = jax.nn.sigmoid(jnp.sum(r, axis=1, keepdims=True))
        wait_all(wg_v, wsem.at[WG_SEM])
        g = _dot_nt(h2b, wg_v[...])
        wait_all(wu_v, wsem.at[WU_SEM])
        u = _dot_nt(h2b, wu_v[...])
        act = (jax.nn.silu(g) * u).astype(bf16)
        out = x1 + gb * (h2 + h2 * 0.0)
        y_scale = gb * r_gate
        for i, (lo, hi) in enumerate(wd_rows):
            wait_all(wd_v.at[lo:hi], wsem.at[WD_SEM + i])
            out = out + y_scale * _dot(act[:, lo:hi], wd_v[lo:hi, :])
        out_ref[...] = out.astype(out_ref.dtype)

    hbm = pl.BlockSpec(memory_space=pltpu.HBM)
    out = pl.pallas_call(
        kernel,
        in_specs=[hbm] * 11,
        out_specs=pl.BlockSpec(memory_space=pltpu.VMEM),
        out_shape=jax.ShapeDtypeStruct((B, D), A_x.dtype),
        scratch_shapes=[
            pltpu.VMEM((N_SLOTS, HG, SEGS, seg, DH), bf16),
            pltpu.VMEM((N_SLOTS, HG, SEGS, seg, DH), bf16),
            pltpu.VMEM((4, D // 4, H * DH), bf16),
            pltpu.VMEM((4, H * DH // 4, D), bf16),
            pltpu.VMEM((4, D // 4, 6 * D), bf16),
            pltpu.VMEM((F, D), bf16),
            pltpu.VMEM((F, D), bf16),
            pltpu.VMEM((F, D), bf16),
            pltpu.VMEM((B, D), bf16),
            pltpu.VMEM((B, D), bf16),
            pltpu.VMEM((D // LANES, LANES), bf16),
            pltpu.VMEM((H, B, DH), bf16),
            pltpu.VMEM((H, B, DH), f32),
            pltpu.SemaphoreType.DMA((N_SLOTS,)),
            pltpu.SemaphoreType.DMA((N_SLOTS,)),
            pltpu.SemaphoreType.DMA((8 + len(wd_rows),)),
        ],
        compiler_params=pltpu.CompilerParams(
            vmem_limit_bytes=100 * 1024 * 1024,
            disable_bounds_checks=True,
            disable_semaphore_checks=True,
        ),
    )(
        A_x.reshape(B, D),
        A_k_cache.reshape(B, H * SEGS, seg, DH),
        A_v_cache.reshape(B, H * SEGS, seg, DH),
        A_wq.reshape(4, D // 4, H * DH),
        A_wo.reshape(4, H * DH // 4, D),
        B_w_r.reshape(D // LANES, LANES),
        B_w_gate.T,
        B_w_up.T,
        B_w_down,
        c,
        w_mod.reshape(4, D // 4, 6 * D),
    )
    return out.reshape(B, SQ, D)
```

```python
import jax
import jax.numpy as jnp
from jax import lax
import jax.experimental.pallas as pl
import jax.experimental.pallas.tpu as pltpu

f32 = jnp.float32
bf16 = jnp.bfloat16
LANES = 128
EPS = 1e-5
NT_DIMS = (((1,), (1,)), ((), ()))

HG = 4
SEGS = 2
ROWS = 128
N_SLOTS = 3
AHEAD = 8
TAIL_FIRST, TAIL_STEP = 64, 28


def _layernorm(x):
    xc = x - jnp.mean(x, axis=-1, keepdims=True)
    var = jnp.mean(xc * xc, axis=-1, keepdims=True)
    return xc / jnp.sqrt(var + EPS)


def _dot(a, w):
    return jnp.dot(a, w, preferred_element_type=f32)


def _dot_nt(a, w):
    return lax.dot_general(a, w, NT_DIMS, preferred_element_type=f32)


@jax.jit
def pallas_adaLN_cond__gqa_block_cached__moe_arch_mod__decode_kernel(
    A_x: jax.Array,
    A_k_cache: jax.Array,
    A_v_cache: jax.Array,
    A_wq: jax.Array,
    A_wo: jax.Array,
    B_x: jax.Array,
    B_w_r: jax.Array,
    B_w_gate: jax.Array,
    B_w_up: jax.Array,
    B_w_down: jax.Array,
    c: jax.Array,
    w_mod: jax.Array,
):
    del B_x
    B, SQ, D = A_x.shape
    _, H, SK, DH = A_k_cache.shape
    F = B_w_gate.shape[1]
    assert SQ == 1 and A_wq.shape == (D, H * DH) and w_mod.shape == (D, 6 * D)
    assert D % LANES == 0 and DH == LANES
    scale = DH ** -0.5

    seg = SK // SEGS
    n_grp = seg // ROWS
    n_steps = B * H
    n_grp_all = n_steps // HG * n_grp
    grp_step = n_grp // HG
    last_kv_step = -(-(n_grp_all - n_grp - AHEAD) // grp_step) - 1
    assert SK % (SEGS * ROWS) == 0 and H % HG == 0 and n_grp % HG == 0 and AHEAD <= n_grp

    cuts = sorted({0, F, *(LANES * (F // LANES * k // 10) for k in (4, 7, 9))})
    wd_rows = tuple(zip(cuts[:-1], cuts[1:]))

    def kernel(x_hbm, k_hbm, v_hbm, wq_hbm, wo_hbm, wr_hbm, wg_hbm, wu_hbm, wd_hbm, c_hbm, wm_hbm,
               out_ref,
               kbuf, vbuf, wq_v, wo_v, wm_v, wg_v, wu_v, wd_v, x_v, c_v, wr_v, q_v, o_v,
               ksem, vsem, wsem):
        C_SEM, X_SEM, WM_SEM, WQ_SEM, WO_SEM, WR_SEM, WG_SEM, WU_SEM, WD_SEM = range(9)

        def copy(src, dst, sem):
            return pltpu.make_async_copy(src, dst, sem)

        def wait_all(buf, sem):
            copy(buf, buf, sem).wait()

        def kv_issue(lo, hi):
            def group(u, _):
                blk = u // n_grp
                slot, hg, b = blk % N_SLOTS, blk // B, blk % B
                for sg in range(SEGS):
                    rows = pl.ds(pl.multiple_of(sg * seg + u % n_grp * ROWS, ROWS), ROWS)
                    for j in range(HG):
                        h = hg + j * (H // HG)
                        copy(k_hbm.at[b, h, rows], kbuf.at[slot, j, rows], ksem.at[slot]).start(priority=0)
                        copy(v_hbm.at[b, h, rows], vbuf.at[slot, j, rows], vsem.at[slot]).start(priority=1)
            lax.fori_loop(lo, hi, group, None)

        def wide_issue(src, dst, sem):
            def body(i, _):
                rows = pl.ds(pl.multiple_of(i * 8, 8), 8)
                for c0 in range(0, src.shape[2], 8 * LANES):
                    for p in range(2):
                        idx = (slice(2 * p, 2 * p + 2), rows, slice(c0, c0 + 8 * LANES))
                        copy(src.at[idx], dst.at[idx], sem).start(priority=p)
            lax.fori_loop(0, src.shape[1] // 8, body, None)

        tail = []
        for r0 in range(0, wo_hbm.shape[1], 16):
            for p in range(2):
                idx = (slice(2 * p, 2 * p + 2), slice(r0, r0 + 16))
                tail.append((copy(wo_hbm.at[idx], wo_v.at[idx], wsem.at[WO_SEM]), p))
        tail.append((copy(wr_hbm, wr_v, wsem.at[WR_SEM]), 0))
        for r0 in range(0, F, 32):
            rows = slice(r0, min(r0 + 32, F))
            tail.append((copy(wg_hbm.at[rows], wg_v.at[rows], wsem.at[WG_SEM]), 0))
            tail.append((copy(wu_hbm.at[rows], wu_v.at[rows], wsem.at[WU_SEM]), 1))
        for i, (lo, hi) in enumerate(wd_rows):
            for r0 in range(lo, hi, 32):
                rows = slice(r0, min(r0 + 32, hi))
                tail.append((copy(wd_hbm.at[rows], wd_v.at[rows], wsem.at[WD_SEM + i]), r0 // 32 % 2))
        tail_cuts = [0]
        for i in range(n_steps - last_kv_step):
            tail_cuts.append(min(len(tail), tail_cuts[-1] + (TAIL_STEP if i else TAIL_FIRST)))

        def tail_issue(lo, hi):
            for cp, queue in tail[lo:hi]:
                cp.start(priority=queue)

        wide_issue(wm_hbm, wm_v, wsem.at[WM_SEM])
        copy(c_hbm, c_v, wsem.at[C_SEM]).start(priority=0)
        copy(x_hbm, x_v, wsem.at[X_SEM]).start(priority=1)
        wide_issue(wq_hbm, wq_v, wsem.at[WQ_SEM])

        wait_all(wm_v, wsem.at[WM_SEM])
        wait_all(c_v, wsem.at[C_SEM])
        silu_c = jax.nn.silu(c_v[...].astype(f32)).astype(bf16)
        mod = _dot(silu_c, wm_v[...].reshape(D, 6 * D))
        sa, ca, ga, sb, cb, gb = (mod[:, i * D:(i + 1) * D] for i in range(6))
        wait_all(x_v, wsem.at[X_SEM])
        x0 = x_v[...].astype(f32)
        h1 = (_layernorm(x0) * (1 + ca) + sa).astype(bf16)

        kv_issue(0, n_grp // 2)
        o_v[...] = jnp.zeros_like(o_v)

        wait_all(wq_v, wsem.at[WQ_SEM])
        q = _dot(h1, wq_v[...].reshape(D, H * DH)).astype(bf16)
        for h in range(H):
            q_v[h] = q[:, h * DH:(h + 1) * DH]

        kv_issue(n_grp // 2, n_grp + AHEAD)

        batch_row = lax.broadcasted_iota(jnp.int32, (B, DH), 0)

        def head_step(s, _):
            blk, j = s // HG, s % HG
            slot, hg, b = blk % N_SLOTS, blk // B, blk % B
            h = hg + j * (H // HG)

            @pl.when(j == 0)
            def _():
                wait_all(kbuf.at[slot], ksem.at[slot])
                wait_all(vbuf.at[slot], vsem.at[slot])

            scores = _dot_nt(q_v[h], kbuf[slot, j])
            p = jnp.exp((scores - jnp.max(scores, axis=1, keepdims=True)) * scale)
            denom = jnp.sum(p, axis=1, keepdims=True)
            o = _dot(p.astype(bf16), vbuf[slot, j]) / denom
            o_v[h] = jnp.where(batch_row == b, o, o_v[h])

            lo = jnp.minimum(n_grp + AHEAD + grp_step * s, n_grp_all)
            kv_issue(lo, jnp.minimum(lo + grp_step, n_grp_all))

            for i in range(len(tail_cuts) - 1):
                @pl.when(s == last_kv_step + i)
                def _():
                    tail_issue(tail_cuts[i], tail_cuts[i + 1])

        lax.fori_loop(0, n_steps, head_step, None)
        tail_issue(tail_cuts[-1], len(tail))

        wait_all(wo_v, wsem.at[WO_SEM])
        o_all = jnp.concatenate([o_v[h] for h in range(H)], axis=1).astype(bf16)
        x1 = x0 + ga * _dot(o_all, wo_v[...].reshape(H * DH, D))
        h2 = _layernorm(x1) * (1 + cb) + sb
        h2b = h2.astype(bf16)
        wait_all(wr_v, wsem.at[WR_SEM])
        w_r = wr_v[...].astype(f32)
        h2r = h2b.astype(f32)
        r = h2r[:, 0:LANES] * w_r[0:1, :]
        for i in range(1, D // LANES):
            r = r + h2r[:, i * LANES:(i + 1) * LANES] * w_r[i:i + 1, :]
        r_gate = jax.nn.sigmoid(jnp.sum(r, axis=1, keepdims=True))
        wait_all(wg_v, wsem.at[WG_SEM])
        g = _dot_nt(h2b, wg_v[...])
        wait_all(wu_v, wsem.at[WU_SEM])
        u = _dot_nt(h2b, wu_v[...])
        act = (jax.nn.silu(g) * u).astype(bf16)
        out = x1 + gb * (h2 + h2 * 0.0)
        y_scale = gb * r_gate
        for i, (lo, hi) in enumerate(wd_rows):
            wait_all(wd_v.at[lo:hi], wsem.at[WD_SEM + i])
            out = out + y_scale * _dot(act[:, lo:hi], wd_v[lo:hi, :])
        out_ref[...] = out.astype(out_ref.dtype)

    hbm = pl.BlockSpec(memory_space=pltpu.HBM)
    out = pl.pallas_call(
        kernel,
        in_specs=[hbm] * 11,
        out_specs=pl.BlockSpec(memory_space=pltpu.VMEM),
        out_shape=jax.ShapeDtypeStruct((B, D), A_x.dtype),
        scratch_shapes=[
            pltpu.VMEM((N_SLOTS, HG, SK, DH), bf16),
            pltpu.VMEM((N_SLOTS, HG, SK, DH), bf16),
            pltpu.VMEM((4, D // 4, H * DH), bf16),
            pltpu.VMEM((4, H * DH // 4, D), bf16),
            pltpu.VMEM((4, D // 4, 6 * D), bf16),
            pltpu.VMEM((F, D), bf16),
            pltpu.VMEM((F, D), bf16),
            pltpu.VMEM((F, D), bf16),
            pltpu.VMEM((B, D), bf16),
            pltpu.VMEM((B, D), bf16),
            pltpu.VMEM((D // LANES, LANES), bf16),
            pltpu.VMEM((H, B, DH), bf16),
            pltpu.VMEM((H, B, DH), f32),
            pltpu.SemaphoreType.DMA((N_SLOTS,)),
            pltpu.SemaphoreType.DMA((N_SLOTS,)),
            pltpu.SemaphoreType.DMA((8 + len(wd_rows),)),
        ],
        compiler_params=pltpu.CompilerParams(
            vmem_limit_bytes=100 * 1024 * 1024,
            disable_semaphore_checks=True,
        ),
    )(
        A_x.reshape(B, D),
        A_k_cache,
        A_v_cache,
        A_wq.reshape(4, D // 4, H * DH),
        A_wo.reshape(4, H * DH // 4, D),
        B_w_r.reshape(D // LANES, LANES),
        B_w_gate.T,
        B_w_up.T,
        B_w_down,
        c,
        w_mod.reshape(4, D // 4, 6 * D),
    )
    return out.reshape(B, SQ, D)
```

```python
import jax
import jax.numpy as jnp
from jax import lax
import jax.experimental.pallas as pl
import jax.experimental.pallas.tpu as pltpu

f32 = jnp.float32
bf16 = jnp.bfloat16
LANES = 128
EPS = 1e-5
NT_DIMS = (((1,), (1,)), ((), ()))

HG = 4
SEGS = 2
ROWS = 64
V_SKEW = 1
N_SLOTS = 3
AHEAD = 16
TAIL_FIRST, TAIL_STEP = 64, 28


def _layernorm(x):
    xc = x - jnp.mean(x, axis=-1, keepdims=True)
    var = jnp.mean(xc * xc, axis=-1, keepdims=True)
    return xc / jnp.sqrt(var + EPS)


def _dot(a, w):
    return jnp.dot(a, w, preferred_element_type=f32)


def _dot_nt(a, w):
    return lax.dot_general(a, w, NT_DIMS, preferred_element_type=f32)


@jax.jit
def pallas_adaLN_cond__gqa_block_cached__moe_arch_mod__decode_kernel(
    A_x: jax.Array,
    A_k_cache: jax.Array,
    A_v_cache: jax.Array,
    A_wq: jax.Array,
    A_wo: jax.Array,
    B_x: jax.Array,
    B_w_r: jax.Array,
    B_w_gate: jax.Array,
    B_w_up: jax.Array,
    B_w_down: jax.Array,
    c: jax.Array,
    w_mod: jax.Array,
):
    del B_x
    B, SQ, D = A_x.shape
    _, H, SK, DH = A_k_cache.shape
    F = B_w_gate.shape[1]
    assert SQ == 1 and A_wq.shape == (D, H * DH) and w_mod.shape == (D, 6 * D)
    assert D % LANES == 0 and DH == LANES
    scale = DH ** -0.5

    seg = SK // SEGS
    n_grp = seg // ROWS
    n_steps = B * H
    n_grp_all = n_steps // HG * n_grp
    grp_step = n_grp // HG
    last_kv_step = -(-(n_grp_all - n_grp - AHEAD) // grp_step) - 1
    assert SK % (SEGS * ROWS) == 0 and H % HG == 0 and n_grp % HG == 0 and AHEAD <= n_grp

    cuts = sorted({0, F, *(LANES * (F // LANES * k // 10) for k in (4, 7, 9))})
    wd_rows = tuple(zip(cuts[:-1], cuts[1:]))

    def kernel(x_hbm, k_hbm, v_hbm, wq_hbm, wo_hbm, wr_hbm, wg_hbm, wu_hbm, wd_hbm, c_hbm, wm_hbm,
               out_ref,
               kbuf, vbuf, wq_v, wo_v, wm_v, wg_v, wu_v, wd_v, x_v, c_v, wr_v, q_v, o_v,
               ksem, vsem, wsem):
        C_SEM, X_SEM, WM_SEM, WQ_SEM, WO_SEM, WR_SEM, WG_SEM, WU_SEM, WD_SEM = range(9)

        def copy(src, dst, sem):
            return pltpu.make_async_copy(src, dst, sem)

        def wait_all(buf, sem):
            copy(buf, buf, sem).wait()

        def kv_issue(lo, hi):
            def group(u, _):
                blk = u // n_grp
                slot, hg, b = blk % N_SLOTS, blk // B, blk % B
                k_rows = pl.ds(pl.multiple_of(u % n_grp * ROWS, ROWS), ROWS)
                v_rows = pl.ds(pl.multiple_of((u + V_SKEW) % n_grp * ROWS, ROWS), ROWS)
                for j in range(HG):
                    segs = pl.ds((hg * HG + j) * SEGS, SEGS)
                    copy(k_hbm.at[b, segs, k_rows], kbuf.at[slot, j, :, k_rows],
                         ksem.at[slot]).start(priority=0)
                    copy(v_hbm.at[b, segs, v_rows], vbuf.at[slot, j, :, v_rows],
                         vsem.at[slot]).start(priority=1)
            lax.fori_loop(lo, hi, group, None)

        def wide_issue(src, dst, sem):
            def body(i, _):
                rows = pl.ds(pl.multiple_of(i * 8, 8), 8)
                for c0 in range(0, src.shape[2], 8 * LANES):
                    for p in range(2):
                        idx = (slice(2 * p, 2 * p + 2), rows, slice(c0, c0 + 8 * LANES))
                        copy(src.at[idx], dst.at[idx], sem).start(priority=p)
            lax.fori_loop(0, src.shape[1] // 8, body, None)

        tail = []
        for r0 in range(0, wo_hbm.shape[1], 16):
            for p in range(2):
                idx = (slice(2 * p, 2 * p + 2), slice(r0, r0 + 16))
                tail.append((copy(wo_hbm.at[idx], wo_v.at[idx], wsem.at[WO_SEM]), p))
        tail.append((copy(wr_hbm, wr_v, wsem.at[WR_SEM]), 0))
        for r0 in range(0, F, 32):
            rows = slice(r0, min(r0 + 32, F))
            tail.append((copy(wg_hbm.at[rows], wg_v.at[rows], wsem.at[WG_SEM]), 0))
            tail.append((copy(wu_hbm.at[rows], wu_v.at[rows], wsem.at[WU_SEM]), 1))
        for i, (lo, hi) in enumerate(wd_rows):
            for r0 in range(lo, hi, 32):
                rows = slice(r0, min(r0 + 32, hi))
                tail.append((copy(wd_hbm.at[rows], wd_v.at[rows], wsem.at[WD_SEM + i]), r0 // 32 % 2))
        tail_cuts = [0]
        for i in range(n_steps - last_kv_step):
            tail_cuts.append(min(len(tail), tail_cuts[-1] + (TAIL_STEP if i else TAIL_FIRST)))

        def tail_issue(lo, hi):
            for cp, queue in tail[lo:hi]:
                cp.start(priority=queue)

        wide_issue(wm_hbm, wm_v, wsem.at[WM_SEM])
        copy(c_hbm, c_v, wsem.at[C_SEM]).start(priority=0)
        copy(x_hbm, x_v, wsem.at[X_SEM]).start(priority=1)
        wide_issue(wq_hbm, wq_v, wsem.at[WQ_SEM])

        wait_all(wm_v, wsem.at[WM_SEM])
        wait_all(c_v, wsem.at[C_SEM])
        silu_c = jax.nn.silu(c_v[...].astype(f32)).astype(bf16)
        mod = _dot(silu_c, wm_v[...].reshape(D, 6 * D))
        sa, ca, ga, sb, cb, gb = (mod[:, i * D:(i + 1) * D] for i in range(6))
        wait_all(x_v, wsem.at[X_SEM])
        x0 = x_v[...].astype(f32)
        h1 = (_layernorm(x0) * (1 + ca) + sa).astype(bf16)

        kv_issue(0, n_grp // 2)
        o_v[...] = jnp.zeros_like(o_v)

        wait_all(wq_v, wsem.at[WQ_SEM])
        q = _dot(h1, wq_v[...].reshape(D, H * DH)).astype(bf16)
        for h in range(H):
            q_v[h] = q[:, h * DH:(h + 1) * DH]

        kv_issue(n_grp // 2, n_grp + AHEAD)

        batch_row = lax.broadcasted_iota(jnp.int32, (B, DH), 0)

        def head_step(s, _):
            blk, j = s // HG, s % HG
            slot, hg, b = blk % N_SLOTS, blk // B, blk % B
            h = hg * HG + j

            @pl.when(j == 0)
            def _():
                wait_all(kbuf.at[slot], ksem.at[slot])
                wait_all(vbuf.at[slot], vsem.at[slot])

            scores = _dot_nt(q_v[h], kbuf[slot, j].reshape(SK, DH))
            p = jnp.exp((scores - jnp.max(scores, axis=1, keepdims=True)) * scale)
            denom = jnp.sum(p, axis=1, keepdims=True)
            o = _dot(p.astype(bf16), vbuf[slot, j].reshape(SK, DH)) / denom
            o_v[h] = jnp.where(batch_row == b, o, o_v[h])

            lo = jnp.minimum(n_grp + AHEAD + grp_step * s, n_grp_all)
            kv_issue(lo, jnp.minimum(lo + grp_step, n_grp_all))

            for i in range(len(tail_cuts) - 1):
                @pl.when(s == last_kv_step + i)
                def _():
                    tail_issue(tail_cuts[i], tail_cuts[i + 1])

        lax.fori_loop(0, n_steps, head_step, None)
        tail_issue(tail_cuts[-1], len(tail))

        wait_all(wo_v, wsem.at[WO_SEM])
        o_all = jnp.concatenate([o_v[h] for h in range(H)], axis=1).astype(bf16)
        x1 = x0 + ga * _dot(o_all, wo_v[...].reshape(H * DH, D))
        h2 = _layernorm(x1) * (1 + cb) + sb
        h2b = h2.astype(bf16)
        wait_all(wr_v, wsem.at[WR_SEM])
        w_r = wr_v[...].astype(f32)
        h2r = h2b.astype(f32)
        r = h2r[:, 0:LANES] * w_r[0:1, :]
        for i in range(1, D // LANES):
            r = r + h2r[:, i * LANES:(i + 1) * LANES] * w_r[i:i + 1, :]
        r_gate = jax.nn.sigmoid(jnp.sum(r, axis=1, keepdims=True))
        wait_all(wg_v, wsem.at[WG_SEM])
        g = _dot_nt(h2b, wg_v[...])
        wait_all(wu_v, wsem.at[WU_SEM])
        u = _dot_nt(h2b, wu_v[...])
        act = (jax.nn.silu(g) * u).astype(bf16)
        out = x1 + gb * (h2 + h2 * 0.0)
        y_scale = gb * r_gate
        for i, (lo, hi) in enumerate(wd_rows):
            wait_all(wd_v.at[lo:hi], wsem.at[WD_SEM + i])
            out = out + y_scale * _dot(act[:, lo:hi], wd_v[lo:hi, :])
        out_ref[...] = out.astype(out_ref.dtype)

    hbm = pl.BlockSpec(memory_space=pltpu.HBM)
    out = pl.pallas_call(
        kernel,
        in_specs=[hbm] * 11,
        out_specs=pl.BlockSpec(memory_space=pltpu.VMEM),
        out_shape=jax.ShapeDtypeStruct((B, D), A_x.dtype),
        scratch_shapes=[
            pltpu.VMEM((N_SLOTS, HG, SEGS, seg, DH), bf16),
            pltpu.VMEM((N_SLOTS, HG, SEGS, seg, DH), bf16),
            pltpu.VMEM((4, D // 4, H * DH), bf16),
            pltpu.VMEM((4, H * DH // 4, D), bf16),
            pltpu.VMEM((4, D // 4, 6 * D), bf16),
            pltpu.VMEM((F, D), bf16),
            pltpu.VMEM((F, D), bf16),
            pltpu.VMEM((F, D), bf16),
            pltpu.VMEM((B, D), bf16),
            pltpu.VMEM((B, D), bf16),
            pltpu.VMEM((D // LANES, LANES), bf16),
            pltpu.VMEM((H, B, DH), bf16),
            pltpu.VMEM((H, B, DH), f32),
            pltpu.SemaphoreType.DMA((N_SLOTS,)),
            pltpu.SemaphoreType.DMA((N_SLOTS,)),
            pltpu.SemaphoreType.DMA((8 + len(wd_rows),)),
        ],
        compiler_params=pltpu.CompilerParams(
            vmem_limit_bytes=100 * 1024 * 1024,
            disable_semaphore_checks=True,
        ),
    )(
        A_x.reshape(B, D),
        A_k_cache.reshape(B, H * SEGS, seg, DH),
        A_v_cache.reshape(B, H * SEGS, seg, DH),
        A_wq.reshape(4, D // 4, H * DH),
        A_wo.reshape(4, H * DH // 4, D),
        B_w_r.reshape(D // LANES, LANES),
        B_w_gate.T,
        B_w_up.T,
        B_w_down,
        c,
        w_mod.reshape(4, D // 4, 6 * D),
    )
    return out.reshape(B, SQ, D)
```

```python
import jax
import jax.numpy as jnp
from jax import lax
import jax.experimental.pallas as pl
import jax.experimental.pallas.tpu as pltpu

f32 = jnp.float32
bf16 = jnp.bfloat16
LANES = 128
EPS = 1e-5
NT_DIMS = (((1,), (1,)), ((), ()))

HG = 4
SEGS = 2
ROWS = 64
N_SLOTS = 3
AHEAD = 24
TAIL_FIRST, TAIL_STEP = 64, 28


def _layernorm(x):
    xc = x - jnp.mean(x, axis=-1, keepdims=True)
    var = jnp.mean(xc * xc, axis=-1, keepdims=True)
    return xc / jnp.sqrt(var + EPS)


def _dot(a, w):
    return jnp.dot(a, w, preferred_element_type=f32)


def _dot_nt(a, w):
    return lax.dot_general(a, w, NT_DIMS, preferred_element_type=f32)


@jax.jit
def pallas_adaLN_cond__gqa_block_cached__moe_arch_mod__decode_kernel(
    A_x: jax.Array,
    A_k_cache: jax.Array,
    A_v_cache: jax.Array,
    A_wq: jax.Array,
    A_wo: jax.Array,
    B_x: jax.Array,
    B_w_r: jax.Array,
    B_w_gate: jax.Array,
    B_w_up: jax.Array,
    B_w_down: jax.Array,
    c: jax.Array,
    w_mod: jax.Array,
):
    del B_x
    B, SQ, D = A_x.shape
    _, H, SK, DH = A_k_cache.shape
    F = B_w_gate.shape[1]
    assert SQ == 1 and A_wq.shape == (D, H * DH) and w_mod.shape == (D, 6 * D)
    assert D % LANES == 0 and DH == LANES
    scale = DH ** -0.5

    seg = SK // SEGS
    n_grp = seg // ROWS
    n_steps = B * H
    n_grp_all = n_steps // HG * n_grp
    grp_step = n_grp // HG
    last_kv_step = -(-(n_grp_all - n_grp - AHEAD) // grp_step) - 1
    assert SK % (SEGS * ROWS) == 0 and H % HG == 0 and n_grp % HG == 0 and AHEAD <= n_grp

    cuts = sorted({0, F, *(LANES * (F // LANES * k // 10) for k in (4, 7, 9))})
    wd_rows = tuple(zip(cuts[:-1], cuts[1:]))

    def kernel(x_hbm, k_hbm, v_hbm, wq_hbm, wo_hbm, wr_hbm, wg_hbm, wu_hbm, wd_hbm, c_hbm, wm_hbm,
               out_ref,
               kbuf, vbuf, wq_v, wo_v, wm_v, wg_v, wu_v, wd_v, x_v, c_v, wr_v, q_v, o_v,
               ksem, vsem, wsem):
        C_SEM, X_SEM, WM_SEM, WQ_SEM, WO_SEM, WR_SEM, WG_SEM, WU_SEM, WD_SEM = range(9)

        def copy(src, dst, sem):
            return pltpu.make_async_copy(src, dst, sem)

        def wait_all(buf, sem):
            copy(buf, buf, sem).wait()

        def kv_issue(lo, hi):
            def group(u, _):
                blk = u // n_grp
                slot, hg, b = blk % N_SLOTS, blk // B, blk % B
                rows = pl.ds(pl.multiple_of(u % n_grp * ROWS, ROWS), ROWS)
                for j in range(HG):
                    segs = pl.ds((hg * HG + j) * SEGS, SEGS)
                    copy(k_hbm.at[b, segs, rows], kbuf.at[slot, j, :, rows], ksem.at[slot]).start(priority=0)
                    copy(v_hbm.at[b, segs, rows], vbuf.at[slot, j, :, rows], vsem.at[slot]).start(priority=1)
            lax.fori_loop(lo, hi, group, None)

        def wide_issue(src, dst, sem):
            def body(i, _):
                rows = pl.ds(pl.multiple_of(i * 8, 8), 8)
                for c0 in range(0, src.shape[2], 8 * LANES):
                    for p in range(2):
                        idx = (slice(2 * p, 2 * p + 2), rows, slice(c0, c0 + 8 * LANES))
                        copy(src.at[idx], dst.at[idx], sem).start(priority=p)
            lax.fori_loop(0, src.shape[1] // 8, body, None)

        tail = []
        for r0 in range(0, wo_hbm.shape[1], 16):
            for p in range(2):
                idx = (slice(2 * p, 2 * p + 2), slice(r0, r0 + 16))
                tail.append((copy(wo_hbm.at[idx], wo_v.at[idx], wsem.at[WO_SEM]), p))
        tail.append((copy(wr_hbm, wr_v, wsem.at[WR_SEM]), 0))
        for r0 in range(0, F, 32):
            rows = slice(r0, min(r0 + 32, F))
            tail.append((copy(wg_hbm.at[rows], wg_v.at[rows], wsem.at[WG_SEM]), 0))
            tail.append((copy(wu_hbm.at[rows], wu_v.at[rows], wsem.at[WU_SEM]), 1))
        for i, (lo, hi) in enumerate(wd_rows):
            for r0 in range(lo, hi, 32):
                rows = slice(r0, min(r0 + 32, hi))
                tail.append((copy(wd_hbm.at[rows], wd_v.at[rows], wsem.at[WD_SEM + i]), r0 // 32 % 2))
        tail_cuts = [0]
        for i in range(n_steps - last_kv_step):
            tail_cuts.append(min(len(tail), tail_cuts[-1] + (TAIL_STEP if i else TAIL_FIRST)))

        def tail_issue(lo, hi):
            for cp, queue in tail[lo:hi]:
                cp.start(priority=queue)

        wide_issue(wm_hbm, wm_v, wsem.at[WM_SEM])
        copy(c_hbm, c_v, wsem.at[C_SEM]).start(priority=0)
        copy(x_hbm, x_v, wsem.at[X_SEM]).start(priority=1)
        wide_issue(wq_hbm, wq_v, wsem.at[WQ_SEM])

        wait_all(wm_v, wsem.at[WM_SEM])
        wait_all(c_v, wsem.at[C_SEM])
        silu_c = jax.nn.silu(c_v[...].astype(f32)).astype(bf16)
        mod = _dot(silu_c, wm_v[...].reshape(D, 6 * D))
        sa, ca, ga, sb, cb, gb = (mod[:, i * D:(i + 1) * D] for i in range(6))
        wait_all(x_v, wsem.at[X_SEM])
        x0 = x_v[...].astype(f32)
        h1 = (_layernorm(x0) * (1 + ca) + sa).astype(bf16)

        kv_issue(0, n_grp // 2)
        o_v[...] = jnp.zeros_like(o_v)

        wait_all(wq_v, wsem.at[WQ_SEM])
        q = _dot(h1, wq_v[...].reshape(D, H * DH)).astype(bf16)
        for h in range(H):
            q_v[h] = q[:, h * DH:(h + 1) * DH]

        kv_issue(n_grp // 2, n_grp + AHEAD)

        batch_row = lax.broadcasted_iota(jnp.int32, (B, DH), 0)

        def head_step(s, _):
            blk, j = s // HG, s % HG
            slot, hg, b = blk % N_SLOTS, blk // B, blk % B
            h = hg * HG + j

            @pl.when(j == 0)
            def _():
                wait_all(kbuf.at[slot], ksem.at[slot])
                wait_all(vbuf.at[slot], vsem.at[slot])

            scores = _dot_nt(q_v[h], kbuf[slot, j].reshape(SK, DH))
            p = jnp.exp((scores - jnp.max(scores, axis=1, keepdims=True)) * scale)
            denom = jnp.sum(p, axis=1, keepdims=True)
            o = _dot(p.astype(bf16), vbuf[slot, j].reshape(SK, DH)) / denom
            o_v[h] = jnp.where(batch_row == b, o, o_v[h])

            lo = jnp.minimum(n_grp + AHEAD + grp_step * s, n_grp_all)
            kv_issue(lo, jnp.minimum(lo + grp_step, n_grp_all))

            for i in range(len(tail_cuts) - 1):
                @pl.when(s == last_kv_step + i)
                def _():
                    tail_issue(tail_cuts[i], tail_cuts[i + 1])

        lax.fori_loop(0, n_steps, head_step, None)
        tail_issue(tail_cuts[-1], len(tail))

        wait_all(wo_v, wsem.at[WO_SEM])
        o_all = jnp.concatenate([o_v[h] for h in range(H)], axis=1).astype(bf16)
        x1 = x0 + ga * _dot(o_all, wo_v[...].reshape(H * DH, D))
        h2 = _layernorm(x1) * (1 + cb) + sb
        h2b = h2.astype(bf16)
        wait_all(wr_v, wsem.at[WR_SEM])
        w_r = wr_v[...].astype(f32)
        h2r = h2b.astype(f32)
        r = h2r[:, 0:LANES] * w_r[0:1, :]
        for i in range(1, D // LANES):
            r = r + h2r[:, i * LANES:(i + 1) * LANES] * w_r[i:i + 1, :]
        r_gate = jax.nn.sigmoid(jnp.sum(r, axis=1, keepdims=True))
        wait_all(wg_v, wsem.at[WG_SEM])
        g = _dot_nt(h2b, wg_v[...])
        wait_all(wu_v, wsem.at[WU_SEM])
        u = _dot_nt(h2b, wu_v[...])
        act = (jax.nn.silu(g) * u).astype(bf16)
        out = x1 + gb * (h2 + h2 * 0.0)
        y_scale = gb * r_gate
        for i, (lo, hi) in enumerate(wd_rows):
            wait_all(wd_v.at[lo:hi], wsem.at[WD_SEM + i])
            out = out + y_scale * _dot(act[:, lo:hi], wd_v[lo:hi, :])
        out_ref[...] = out.astype(out_ref.dtype)

    hbm = pl.BlockSpec(memory_space=pltpu.HBM)
    out = pl.pallas_call(
        kernel,
        in_specs=[hbm] * 11,
        out_specs=pl.BlockSpec(memory_space=pltpu.VMEM),
        out_shape=jax.ShapeDtypeStruct((B, D), A_x.dtype),
        scratch_shapes=[
            pltpu.VMEM((N_SLOTS, HG, SEGS, seg, DH), bf16),
            pltpu.VMEM((N_SLOTS, HG, SEGS, seg, DH), bf16),
            pltpu.VMEM((4, D // 4, H * DH), bf16),
            pltpu.VMEM((4, H * DH // 4, D), bf16),
            pltpu.VMEM((4, D // 4, 6 * D), bf16),
            pltpu.VMEM((F, D), bf16),
            pltpu.VMEM((F, D), bf16),
            pltpu.VMEM((F, D), bf16),
            pltpu.VMEM((B, D), bf16),
            pltpu.VMEM((B, D), bf16),
            pltpu.VMEM((D // LANES, LANES), bf16),
            pltpu.VMEM((H, B, DH), bf16),
            pltpu.VMEM((H, B, DH), f32),
            pltpu.SemaphoreType.DMA((N_SLOTS,)),
            pltpu.SemaphoreType.DMA((N_SLOTS,)),
            pltpu.SemaphoreType.DMA((8 + len(wd_rows),)),
        ],
        compiler_params=pltpu.CompilerParams(
            vmem_limit_bytes=100 * 1024 * 1024,
            disable_semaphore_checks=True,
        ),
    )(
        A_x.reshape(B, D),
        A_k_cache.reshape(B, H * SEGS, seg, DH),
        A_v_cache.reshape(B, H * SEGS, seg, DH),
        A_wq.reshape(4, D // 4, H * DH),
        A_wo.reshape(4, H * DH // 4, D),
        B_w_r.reshape(D // LANES, LANES),
        B_w_gate.T,
        B_w_up.T,
        B_w_down,
        c,
        w_mod.reshape(4, D // 4, 6 * D),
    )
    return out.reshape(B, SQ, D)
```
